```python
import jax
import jax.numpy as jnp

def _softmax(x, axis=-1):
    return jax.nn.softmax(x, axis=axis)
def _gelu(x):
    return jax.nn.gelu(x, approximate=True)
def _silu(x):
    return jax.nn.silu(x)
def _sigmoid(x):
    return jax.nn.sigmoid(x)
def _layernorm(x, axis=-1, eps=1e-5):
    m = jnp.mean(x, axis=axis, keepdims=True)
    v = jnp.var(x, axis=axis, keepdims=True)
    return (x - m) / jnp.sqrt(v + eps)
def _scatter_add(tgt, idx, src, axis=0):
    return tgt.at[idx].add(src)
def _segment_sum(src, seg, n):
    return jax.ops.segment_sum(src, seg, n)
class _Rng:
    def __init__(self, key):
        self._k = key
    def _next(self):
        self._k, sub = jax.random.split(self._k)
        return sub
    def normal(self, shape):
        return jax.random.normal(self._next(), shape, dtype=jnp.bfloat16)
    def randint(self, lo, hi, shape):
        return jax.random.randint(self._next(), shape, lo, hi, dtype=jnp.int32)
    def uniform(self, shape, lo=0.0, hi=1.0):
        return jax.random.uniform(self._next(), shape, jnp.bfloat16, lo, hi)
    def permutation(self, n):
        return jax.random.permutation(self._next(), n)


kernel_name = 'interleave_layers__sliding_block_cached__dense_activation_gelu__decode'

def setup_inputs():
    _rng = _Rng(jax.random.key(int.from_bytes(__import__("os").urandom(4), "little")))
    _w = (lambda a: (lambda t: t.astype(jnp.bfloat16) if jnp.issubdtype(t.dtype, jnp.floating) else t)(jnp.asarray(a)))
    def _A_setup():
        B, Sq, D = 1, 1, 640
        Hq, Hkv, Sk, Dh = 32, 32, 32768, 192
        assert Hq % Hkv == 0, (Hq, Hkv)
        return {
            "x": _w((lambda *s: _rng.normal(s) * 0.05)(B, Sq, D)),
            "k_cache": _w((lambda *s: _rng.normal(s) * 0.05)(B, Hkv, Sk, Dh)),
            "v_cache": _w((lambda *s: _rng.normal(s) * 0.05)(B, Hkv, Sk, Dh)),
            "wq": _w((lambda *s: _rng.normal(s) * 0.05)(D, Hq * Dh) * (D ** -0.5)),
            "wo": _w((lambda *s: _rng.normal(s) * 0.05)(Hq * Dh, D) * ((Hq * Dh) ** -0.5)),
        }
    _A_in = _A_setup()

    def _B_setup():
        B, S, D, F = 1, 1, 640, 1536
        return {
            "x": _w((lambda *s: _rng.normal(s) * 0.05)(B, S, D)),
            "w1": _w((lambda *s: _rng.normal(s) * 0.05)(D, F) * (D ** -0.5)),
            "b1": _w((lambda *s: _rng.normal(s) * 0.05)(F) * 0.01),
            "w2": _w((lambda *s: _rng.normal(s) * 0.05)(F, D) * (F ** -0.5)),
            "b2": _w((lambda *s: _rng.normal(s) * 0.05)(D) * 0.01),
        }
    _B_in = _B_setup()

    return {
        "A_x": _A_in["x"],
        "A_k_cache": _A_in["k_cache"],
        "A_v_cache": _A_in["v_cache"],
        "A_wq": _A_in["wq"],
        "A_wo": _A_in["wo"],
        "B_x": _B_in["x"],
        "B_w1": _B_in["w1"],
        "B_b1": _B_in["b1"],
        "B_w2": _B_in["w2"],
        "B_b2": _B_in["b2"],
    }

def reference(A_x, A_k_cache, A_v_cache, A_wq, A_wo, B_x, B_w1, B_b1, B_w2, B_b2):
    def _A_ref(x, k_cache, v_cache, wq, wo):
        B, Sq, D = x.shape
        Hq, Dh = 32, 192
        Hkv, Sk = k_cache.shape[1], k_cache.shape[2]
        W = min(4096, max(256, Sk // 4))
        rep = Hq // Hkv
        q = (lambda x, *d: x.transpose(*d))((x @ wq).reshape(B, Sq, Hq, Dh), 0, 2, 1, 3)
        k = jnp.repeat(k_cache[:, :, Sk - W:, :], rep, axis=1)
        v = jnp.repeat(v_cache[:, :, Sk - W:, :], rep, axis=1)
        scores = jnp.einsum("bhqd,bhkd->bhqk", q, k) * (Dh ** -0.5)
        p = _softmax(scores, axis=-1)
        o = jnp.einsum("bhqk,bhkd->bhqd", p, v)
        return (lambda x, *d: x.transpose(*d))(o, 0, 2, 1, 3).reshape(B, Sq, Hq * Dh) @ wo

    def _B_ref(x, w1, b1, w2, b2):
        h = jnp.einsum("bsd,df->bsf", x, w1) + b1
        h = _gelu(h)
        return jnp.einsum("bsf,fd->bsd", h, w2) + b2

    x = A_x
    x = x + _A_ref(_layernorm(x, axis=-1), A_k_cache, A_v_cache, A_wq, A_wo)
    x = x + _B_ref(_layernorm(x, axis=-1), B_w1, B_b1, B_w2, B_b2)
    x = x + _A_ref(_layernorm(x, axis=-1), A_k_cache, A_v_cache, A_wq, A_wo)
    x = x + _B_ref(_layernorm(x, axis=-1), B_w1, B_b1, B_w2, B_b2)
    return x
```

```python
import jax
import jax.numpy as jnp
import numpy as np
import jax.experimental.pallas as pl
import jax.experimental.pallas.tpu as pltpu

BF = jnp.bfloat16
F32 = jnp.float32
LANES = 128
HQ, DH = 32, 192
HG = 4
G = HQ // HG
R = HG * DH
RT = R // LANES
AHEAD = 2
NSLOT = AHEAD + 1


def _layernorm(x):
    m = jnp.mean(x, axis=-1, keepdims=True)
    c = x - m
    v = jnp.mean(c * c, axis=-1, keepdims=True)
    return c / jnp.sqrt(v + 1e-5)


def _kernel(x_hbm, k_hbm, v_hbm, wq_hbm, wo_hbm, w1_hbm, b1_hbm, w2_hbm, b2_hbm,
            o_ref,
            xb, b1b, b2b, kb, vb, wqb, wob, w1b, w2b,
            x_s, xn_s, q_s, p_s, l_s, on_s, a_s, sems, msem,
            *, sk, w):
    nj = w // LANES
    dt = wob.shape[0]
    ft = w1b.shape[0]
    d = dt * LANES

    def rows(g):
        return pl.ds(pl.multiple_of(g * R, R), R)

    def qtiles(g):
        return pl.ds(g * RT, RT)

    def start_kv(src, dst, g, sem):
        for j in range(nj):
            pltpu.make_async_copy(
                src.at[rows(g), pl.ds(sk - w + j * LANES, LANES)],
                dst.at[j, rows(g)], sem).start()

    def start_wq(g, sem):
        for t in range(RT):
            c = g * RT + t
            pltpu.make_async_copy(
                wq_hbm.at[:, pl.ds(pl.multiple_of(c * LANES, LANES), LANES)],
                wqb.at[c], sem).start()

    def start_wo(g, sem):
        for t in range(dt):
            pltpu.make_async_copy(
                wo_hbm.at[rows(g), pl.ds(t * LANES, LANES)],
                wob.at[t, rows(g)], sem).start()

    def start_cols(src, dst, sem):
        for t in range(dst.shape[0]):
            pltpu.make_async_copy(
                src.at[:, pl.ds(t * LANES, LANES)], dst.at[t], sem).start()

    def wait(buf, sem):
        pltpu.make_async_copy(buf, buf, sem).wait()

    def batch(s, start):
        sem = sems.at[s % NSLOT]
        static = isinstance(s, int)

        def cond(c, fn):
            if static:
                if c:
                    fn()
            else:
                pl.when(c)(fn)

        if start:
            if static and s == 0:
                start_wq(0, sem)
            cond(s < G, lambda: start_kv(k_hbm, kb, s, sem))
            cond(s + 1 < G, lambda: start_wq(s + 1, sem))
            cond((s >= 1) & (s <= G), lambda: start_kv(v_hbm, vb, s - 1, sem))
            cond(s >= 2, lambda: start_wo(s - 2, sem))
        else:
            if static and s == 0:
                wait(wqb.at[qtiles(0)], sem)
            cond(s < G, lambda: wait(kb.at[:, rows(s)], sem))
            cond(s + 1 < G, lambda: wait(wqb.at[qtiles(s + 1)], sem))
            cond((s >= 1) & (s <= G), lambda: wait(vb.at[:, rows(s - 1)], sem))
            cond(s >= 2, lambda: wait(wob.at[:, rows(s - 2)], sem))

    small = [pltpu.make_async_copy(x_hbm, xb, msem.at[0]),
             pltpu.make_async_copy(b1_hbm, b1b, msem.at[0]),
             pltpu.make_async_copy(b2_hbm, b2b, msem.at[0])]
    batch(0, True)
    for c in small:
        c.start()
    for s in range(1, AHEAD + 1):
        batch(s, True)
    for c in small:
        c.wait()
    x_s[...] = jnp.broadcast_to(xb[0].astype(F32), (8, d))

    def head_mask():
        r = jax.lax.broadcasted_iota(jnp.int32, (8, R), 0)
        c = jax.lax.broadcasted_iota(jnp.int32, (8, R), 1)
        return (c >= r * DH) & (c < (r + 1) * DH)

    def q_proj(g):
        xn = xn_s[...].astype(BF)
        q = jnp.concatenate(
            [jnp.dot(xn, wqb[g * RT + t], preferred_element_type=F32)
             for t in range(RT)], axis=1)
        return jnp.where(head_mask(), q, 0.0)

    def k_pass(g, q):
        s = [jnp.dot(q, kb[j, rows(g)], preferred_element_type=F32)
             for j in range(nj)]
        m = s[0]
        for j in range(1, nj):
            m = jnp.maximum(m, s[j])
        m = jnp.max(m, axis=1, keepdims=True)
        p = [jnp.exp((s[j] - m) * (DH ** -0.5)) for j in range(nj)]
        l = p[0]
        for j in range(1, nj):
            l = l + p[j]
        l = jnp.sum(l, axis=1, keepdims=True)
        return p, l

    def v_pass(g):
        accs = []
        for h in range(HG):
            r0 = pl.multiple_of(g * R + h * DH, DH)
            acc = None
            for j in range(nj):
                t = vb[j, pl.ds(r0, DH)].astype(F32) * p_s[j, h:h + 1, :]
                acc = t if acc is None else acc + t
            accs.append(acc)
        acc = jnp.concatenate(accs, axis=0)
        o = jnp.sum(acc.T, axis=0, keepdims=True)
        return jnp.where(head_mask(), o / l_s[:, 0:1], 0.0)

    def o_proj(g):
        o = on_s[...].astype(BF)
        a_s[...] += jnp.concatenate(
            [jnp.dot(o, wob[t, rows(g)], preferred_element_type=F32)
             for t in range(dt)], axis=1)

    def stage(s, do_q, do_k, do_v, do_o):
        if do_o:
            o_proj(s - 2)
        if do_v:
            o = v_pass(s - 1)
        if do_k:
            p, l = k_pass(s, q_s[...].astype(BF))
        if do_q:
            q_s[...] = q_proj(s + 1)
        if do_v:
            on_s[...] = o
        if do_k:
            for j in range(nj):
                p_s[j] = p[j]
            l_s[...] = jnp.broadcast_to(l, l_s.shape)

    def layer(it, carry):
        first = it == 0

        def sync(s):
            @pl.when(first)
            def _():
                batch(s, False)
                if isinstance(s, int):
                    if s + AHEAD + 1 <= G + 1:
                        batch(s + AHEAD + 1, True)
                    if s == G - 1:
                        start_cols(w1_hbm, w1b, msem.at[0])
                        start_cols(w2_hbm, w2b, msem.at[1])
                else:
                    batch(s + AHEAD + 1, True)

        xn_s[...] = _layernorm(x_s[...])
        a_s[...] = jnp.zeros(a_s.shape, F32)
        sync(0)
        q_s[...] = q_proj(0)
        stage(0, True, True, False, False)
        sync(1)
        stage(1, True, True, True, False)

        def mid(s, c):
            sync(s)
            stage(s, True, True, True, True)
            return c
        jax.lax.fori_loop(2, G - 1, mid, 0)
        sync(G - 1)
        stage(G - 1, False, True, True, True)
        sync(G)
        stage(G, False, False, True, True)
        sync(G + 1)
        stage(G + 1, False, False, False, True)

        x = x_s[...] + jnp.sum(a_s[...], axis=0, keepdims=True)
        xn = _layernorm(x).astype(BF)
        pl.when(first)(lambda: wait(w1b, msem.at[0]))
        b1 = b1b[...].astype(F32)
        h = jnp.concatenate(
            [jnp.dot(xn, w1b[t], preferred_element_type=F32) + b1[t:t + 1]
             for t in range(ft)], axis=1)
        h = jax.nn.gelu(h, approximate=True).astype(BF)
        pl.when(first)(lambda: wait(w2b, msem.at[1]))
        b2 = b2b[...].astype(F32)
        y = jnp.concatenate(
            [jnp.dot(h, w2b[t], preferred_element_type=F32) + b2[t:t + 1]
             for t in range(dt)], axis=1)
        x_s[...] = x + y
        return carry

    jax.lax.fori_loop(0, 2, layer, 0)
    o_ref[0] = x_s[0:1, :].astype(o_ref.dtype)


@jax.jit
def pallas_interleave_layers__sliding_block_cached__dense_activation_gelu__decode_kernel(
    A_x: jax.Array,
    A_k_cache: jax.Array,
    A_v_cache: jax.Array,
    A_wq: jax.Array,
    A_wo: jax.Array,
    B_x: jax.Array,
    B_w1: jax.Array,
    B_b1: jax.Array,
    B_w2: jax.Array,
    B_b2: jax.Array,
):
    del B_x
    d = A_x.shape[-1]
    sk = A_k_cache.shape[2]
    f = B_w1.shape[1]
    w = min(4096, max(256, sk // 4))
    nj, dt, ft = w // LANES, d // LANES, f // LANES
    kt = jnp.swapaxes(A_k_cache, 2, 3).reshape(HQ * DH, sk)
    vt = jnp.swapaxes(A_v_cache, 2, 3).reshape(HQ * DH, sk)
    hbm = pl.BlockSpec(memory_space=pltpu.HBM)

    def body(*refs):
        _kernel(*refs, sk=sk, w=w)

    return pl.pallas_call(
        body,
        out_shape=jax.ShapeDtypeStruct(A_x.shape, A_x.dtype),
        in_specs=[hbm] * 9,
        out_specs=pl.BlockSpec(memory_space=pltpu.VMEM),
        scratch_shapes=[
            pltpu.VMEM(A_x.shape, BF),
            pltpu.VMEM((ft, LANES), BF),
            pltpu.VMEM((dt, LANES), BF),
            pltpu.VMEM((nj, HQ * DH, LANES), BF),
            pltpu.VMEM((nj, HQ * DH, LANES), BF),
            pltpu.VMEM((HQ * DH // LANES, d, LANES), BF),
            pltpu.VMEM((dt, HQ * DH, LANES), BF),
            pltpu.VMEM((ft, d, LANES), BF),
            pltpu.VMEM((dt, f, LANES), BF),
            pltpu.VMEM((8, d), F32),
            pltpu.VMEM((8, d), F32),
            pltpu.VMEM((8, R), F32),
            pltpu.VMEM((nj, 8, LANES), F32),
            pltpu.VMEM((8, LANES), F32),
            pltpu.VMEM((8, R), F32),
            pltpu.VMEM((8, d), F32),
            pltpu.SemaphoreType.DMA((NSLOT,)),
            pltpu.SemaphoreType.DMA((2,)),
        ],
        compiler_params=pltpu.CompilerParams(
            vmem_limit_bytes=126 * 1024 * 1024),
    )(A_x, kt, vt, A_wq, A_wo, B_w1, B_b1.reshape(ft, LANES), B_w2,
      B_b2.reshape(dt, LANES))
```

```python
import jax
import jax.numpy as jnp
import numpy as np
import jax.experimental.pallas as pl
import jax.experimental.pallas.tpu as pltpu

BF = jnp.bfloat16
F32 = jnp.float32
I32 = jnp.int32
LANES = 128
HQ, DH = 32, 192
HG = 4
G = HQ // HG
R = HG * DH
RT = R // LANES
NSLOT = 3
PRIO = 0
W2S = 1280
MXU_SHARE = (3, 2, 2, 2, 2, 2, 3, 12)
EXP2_SCALE = float(DH ** -0.5 * np.log2(np.e))


def _layernorm(x):
    m = jnp.mean(x, axis=-1, keepdims=True)
    c = x - m
    v = jnp.mean(c * c, axis=-1, keepdims=True)
    return c / jnp.sqrt(v + 1e-5)


def _lhs(x):
    return jnp.concatenate([x, x], axis=0).astype(BF)


def _dot(a, b, trans=False):
    return jax.lax.dot_general(a, b, (((1,), (1 if trans else 0,)), ((), ())),
                               preferred_element_type=F32)[:8]


def _own_head(x):
    r = jax.lax.broadcasted_iota(I32, (8, R), 0)
    c = jax.lax.broadcasted_iota(I32, (8, R), 1)
    return jnp.where((c >= r * DH) & (c < (r + 1) * DH), x, 0.0)


def _softmax_terms(scores):
    m = scores[0]
    for s in scores[1:]:
        m = jnp.maximum(m, s)
    m = jnp.max(m, axis=1, keepdims=True)
    p = [jnp.exp2((s - m) * EXP2_SCALE) for s in scores]
    l = p[0]
    for pj in p[1:]:
        l = l + pj
    return p, jnp.sum(l, axis=1, keepdims=True)


def _kernel(x_hbm, k_hbm, v_hbm, wq_hbm, wo_hbm, w1_hbm, b1_hbm, w2_hbm, b2_hbm,
            o_ref, xb, b1b, b2b, kw, vw, wqw, wow, w1w, w2w, zero_s, sems, msem,
            *, sk, w):
    nj = w // LANES
    dt = wow.shape[0]
    ft = w1w.shape[0]
    d, f = dt * LANES, ft * LANES
    kb, vb, wqb, wob, w1b, w2b = (r.bitcast(BF) for r in (kw, vw, wqw, wow, w1w, w2w))

    def ld(ref, t, r0=None, n=None):
        return pltpu.bitcast(ref[t] if r0 is None else ref[t, r0 // 2:(r0 + n) // 2], BF)

    def move(start, sem, parts):
        for src, dst, rows, t0, n, c0 in parts:
            if not start:
                whole = dst.at[pl.ds(t0, n), rows]
                pltpu.make_async_copy(whole, whole, sem).wait()
                continue

            def strip(t, pr):
                pltpu.make_async_copy(
                    src.at[rows, pl.ds(pl.multiple_of(c0 + t * LANES, LANES), LANES)],
                    dst.at[t0 + t, rows], sem).start(priority=pr)
            if PRIO and n % 2 == 0:
                @pl.loop(0, n // 2)
                def _(t):
                    strip(2 * t, 0)
                    strip(2 * t + 1, 1)
            else:
                pl.loop(0, n)(lambda t: strip(t, 0))

    def move_group(start, g):
        rows = pl.ds(pl.multiple_of(g * R, R), R)
        move(start, sems.at[g % NSLOT], [
            (wq_hbm, wqb, slice(None), g * RT, RT, g * R),
            (k_hbm, kb, rows, 0, nj, sk - w),
            (v_hbm, vb, rows, 0, nj, sk - w),
            (wo_hbm, wob, rows, 0, dt, 0)])

    def move_mlp(start, i):
        part = [(w1_hbm, w1b, slice(None), 0, ft, 0),
                (w2_hbm, w2b, pl.ds(0, W2S), 0, dt, 0),
                (w2_hbm, w2b, pl.ds(W2S, f - W2S), 0, dt, 0)][i]
        move(start, msem.at[i], [part])

    small = [pltpu.make_async_copy(x_hbm, xb, msem.at[0]),
             pltpu.make_async_copy(b1_hbm, b1b, msem.at[0]),
             pltpu.make_async_copy(b2_hbm, b2b, msem.at[0])]
    move_group(True, 0)
    for c in small:
        c.start()
    pl.loop(1, NSLOT)(lambda g: move_group(True, g))
    for c in small:
        c.wait()
    zero_s[...] = jnp.zeros(zero_s.shape, I32)

    def mlp(x, streaming):
        xn = _lhs(_layernorm(x))
        b1 = b1b[...].astype(F32)
        b2 = b2b[...].astype(F32)
        if streaming:
            move_mlp(False, 0)
        h = jnp.concatenate(
            [_dot(xn, ld(w1w, t)) + b1[t:t + 1] for t in range(ft)], axis=1)
        h = _lhs(jax.nn.gelu(h, approximate=True))
        y = jnp.concatenate([b2[t:t + 1] for t in range(dt)], axis=1)
        cuts = (0, W2S, f) if streaming else (0, f)
        for i, (a, b) in enumerate(zip(cuts, cuts[1:])):
            if streaming:
                move_mlp(False, 1 + i)
            y = y + jnp.concatenate(
                [_dot(h[:, a:b], ld(w2w, t, a, b - a)) for t in range(dt)], axis=1)
        return x + y

    x = jnp.broadcast_to(xb[0].astype(F32), (8, d))
    xn = _lhs(_layernorm(x))

    def stream_group(g, attn):
        move_group(False, g)
        pl.when(g + NSLOT < G)(lambda: move_group(True, g + NSLOT))

        @pl.when(g + NSLOT == G)
        def _():
            for i in range(3):
                move_mlp(True, i)

        half = pl.ds(pl.multiple_of(g * (R // 2), R // 2), R // 2)
        kg, vg, og = kw.at[:, half], vw.at[:, half], wow.at[:, half]
        qg = wqw.at[pl.ds(g * RT, RT)]
        q = _lhs(_own_head(jnp.concatenate(
            [_dot(xn, ld(qg, t)) for t in range(RT)], axis=1)))
        p, l = _softmax_terms([_dot(q, ld(kg, j)) for j in range(nj)])
        o = _dot(_lhs(p[0]), ld(vg, 0), True)
        for j in range(1, nj):
            o = o + _dot(_lhs(p[j]), ld(vg, j), True)
        o = _lhs(_own_head(o / l))
        return attn + jnp.concatenate([_dot(o, ld(og, t)) for t in range(dt)], axis=1)

    attn = jax.lax.fori_loop(0, G, stream_group, jnp.zeros((8, d), F32))
    x = mlp(x + jnp.sum(attn, axis=0, keepdims=True), True)

    xn = _lhs(_layernorm(x))
    never = zero_s[...] != 0
    attn = jnp.zeros((8, d), F32)
    q, soft, pv = {}, {}, {}
    for s in range(-1, G + 2):
        do_q, do_k, do_v, do_o = s + 1 < G, 0 <= s < G, 1 <= s <= G, s >= 2
        cm = MXU_SHARE[s - 1] * nj // 32 if do_v else 0
        lane_sums = []
        if do_v:
            p = soft[s - 1][0]
            for u in range(R // 16):
                h = u * 16 // DH
                terms = [ld(vw, j, (s - 1) * R + u * 16, 16).astype(F32) * p[j][h:h + 1]
                         for j in range(nj - cm)]
                acc = terms[:3]
                for j in range(3, nj - cm):
                    acc[j % 3] = acc[j % 3] + terms[j]
                lane_sums.append((acc[0] + acc[1] + acc[2]).astype(BF))

        mxu_cost = (do_k * nj * R + do_q * RT * d + do_o * (dt + 2) * R + cm * 2 * R) * (
            1.0 if do_k else 0.97)
        done = [0, 0]

        def paced(a, cost):
            upto = min(len(lane_sums), int(len(lane_sums) * done[0] / mxu_cost))
            done[0] += cost
            if upto > done[1]:
                tie = pltpu.bitcast(lane_sums[done[1]], I32)
                for t in lane_sums[done[1] + 1:upto]:
                    tie = tie | pltpu.bitcast(t, I32)
                done[1] = upto
                a = pltpu.bitcast(jnp.where(never, tie, pltpu.bitcast(a, I32)), BF)
            return a

        def dot(a, b, trans=False):
            tiles = range(0, b.shape[0], LANES)
            if trans:
                return jnp.concatenate(
                    [_dot(paced(a, 2 * LANES), b[t:t + LANES], True) for t in tiles], axis=1)
            return _dot(jnp.concatenate(
                [paced(a[:, t:t + LANES], LANES) for t in tiles], axis=1), b)

        def out_proj():
            return jnp.concatenate(
                [dot(o, ld(wow, t, (s - 2) * R, R)) for t in range(dt)], axis=1)

        if do_o:
            o = dot(jnp.ones((16, LANES), BF), pv[s - 2][0], True) + pv[s - 2][1]
            o = _lhs(_own_head(o / soft[s - 2][1]))
        if do_k:
            soft[s] = _softmax_terms([dot(q[s], ld(kw, j, s * R, R)) for j in range(nj)])
        if do_v:
            rest = jnp.zeros((8, R), F32)
            for j in range(nj - cm, nj):
                if do_o and not do_k and j == nj - cm + 2:
                    attn, do_o = attn + out_proj(), False
                rest = rest + dot(_lhs(p[j]), ld(vw, j, (s - 1) * R, R), True)
            pv[s - 1] = (jnp.concatenate(lane_sums, axis=0), rest)
        if do_o:
            attn = attn + out_proj()
        if do_q:
            q[s + 1] = _lhs(_own_head(jnp.concatenate(
                [dot(xn, ld(wqw, (s + 1) * RT + t)) for t in range(RT)], axis=1)))

    x = mlp(x + jnp.sum(attn, axis=0, keepdims=True), False)
    o_ref[0] = x[0:1].astype(o_ref.dtype)


@jax.jit
def pallas_interleave_layers__sliding_block_cached__dense_activation_gelu__decode_kernel(
    A_x: jax.Array,
    A_k_cache: jax.Array,
    A_v_cache: jax.Array,
    A_wq: jax.Array,
    A_wo: jax.Array,
    B_x: jax.Array,
    B_w1: jax.Array,
    B_b1: jax.Array,
    B_w2: jax.Array,
    B_b2: jax.Array,
):
    del B_x
    d = A_x.shape[-1]
    sk = A_k_cache.shape[2]
    f = B_w1.shape[1]
    w = min(4096, max(256, sk // 4))
    nj, dt, ft = w // LANES, d // LANES, f // LANES
    kt = jnp.swapaxes(A_k_cache, 2, 3).reshape(HQ * DH, sk)
    vt = jnp.swapaxes(A_v_cache, 2, 3).reshape(HQ * DH, sk)

    def body(*refs):
        _kernel(*refs, sk=sk, w=w)

    return pl.pallas_call(
        body,
        out_shape=jax.ShapeDtypeStruct(A_x.shape, A_x.dtype),
        in_specs=[pl.BlockSpec(memory_space=pltpu.HBM)] * 9,
        out_specs=pl.BlockSpec(memory_space=pltpu.VMEM),
        scratch_shapes=[
            pltpu.VMEM(A_x.shape, BF),
            pltpu.VMEM((ft, LANES), BF),
            pltpu.VMEM((dt, LANES), BF),
            pltpu.VMEM((nj, HQ * DH // 2 + 8, LANES), I32),
            pltpu.VMEM((nj, HQ * DH // 2 + 8, LANES), I32),
            pltpu.VMEM((HQ * DH // LANES, d // 2, LANES), I32),
            pltpu.VMEM((dt, HQ * DH // 2, LANES), I32),
            pltpu.VMEM((ft, d // 2, LANES), I32),
            pltpu.VMEM((dt, f // 2, LANES), I32),
            pltpu.VMEM((8, LANES), I32),
            pltpu.SemaphoreType.DMA((NSLOT,)),
            pltpu.SemaphoreType.DMA((3,)),
        ],
        compiler_params=pltpu.CompilerParams(vmem_limit_bytes=126 * 1024 * 1024),
    )(A_x, kt, vt, A_wq, A_wo, B_w1, B_b1.reshape(ft, LANES), B_w2,
      B_b2.reshape(dt, LANES))
```

```python
import jax
import jax.numpy as jnp
import numpy as np
import jax.experimental.pallas as pl
import jax.experimental.pallas.tpu as pltpu

BF = jnp.bfloat16
F32 = jnp.float32
I32 = jnp.int32
LANES = 128
HQ, DH = 32, 192
HG = 4
G = HQ // HG
R = HG * DH
RT = R // LANES
NSLOT = 3
PAIR = 0
PAIRQ = 0
NL = 1
TR = 128
STEP = 4
W2S = 1280
MXU_SHARE = (3, 2, 2, 2, 2, 2, 3, 12)
EXP2_SCALE = float(DH ** -0.5 * np.log2(np.e))


def _layernorm(x):
    m = jnp.mean(x, axis=-1, keepdims=True)
    c = x - m
    v = jnp.mean(c * c, axis=-1, keepdims=True)
    return c / jnp.sqrt(v + 1e-5)


def _lhs(x):
    return jnp.concatenate([x, x], axis=0).astype(BF)


def _dot(a, b, trans=False):
    return jax.lax.dot_general(a, b, (((1,), (1 if trans else 0,)), ((), ())),
                               preferred_element_type=F32)[:8]


def _own_head(x):
    r = jax.lax.broadcasted_iota(I32, (8, R), 0)
    c = jax.lax.broadcasted_iota(I32, (8, R), 1)
    return jnp.where((c >= r * DH) & (c < (r + 1) * DH), x, 0.0)


def _softmax_terms(scores):
    m = scores[0]
    for s in scores[1:]:
        m = jnp.maximum(m, s)
    m = jnp.max(m, axis=1, keepdims=True)
    p = [jnp.exp2((s - m) * EXP2_SCALE) for s in scores]
    l = p[0]
    for pj in p[1:]:
        l = l + pj
    return p, jnp.sum(l, axis=1, keepdims=True)


def _kernel(x_hbm, k_hbm, v_hbm, wq_hbm, wo_hbm, w1_hbm, b1_hbm, w2_hbm, b2_hbm,
            o_ref, xb, b1b, b2b, kw, vw, wqw, wow, w1w, w2w, o_s, zero_s, sems, msem,
            *, sk, w):
    nj = w // LANES
    dt = wow.shape[0]
    ft = w1w.shape[0]
    d, f = dt * LANES, ft * LANES
    kb, vb, wqb, wob, w1b, w2b = (r.bitcast(BF) for r in (kw, vw, wqw, wow, w1w, w2w))

    def ld(ref, t, r0=None, n=None):
        return pltpu.bitcast(ref[t] if r0 is None else ref[t, r0 // 2:(r0 + n) // 2], BF)

    def tile(src, dst, r0, i, sem, queue, c0=0):
        r, c = divmod(i, dst.shape[0])
        r = pl.ds(pl.multiple_of(r0 + r * TR, TR), TR)
        pltpu.make_async_copy(src.at[r, pl.ds(c0 + c * LANES, LANES)],
                              dst.at[c, r], sem).start(priority=queue)

    def wait(buf, sem):
        pltpu.make_async_copy(buf, buf, sem).wait()

    def feed_kv(r0, lo, hi, sem):
        for i in range(lo, hi):
            tile(k_hbm, kb, r0, i, sem, 0, sk - w)
            tile(v_hbm, vb, r0, i, sem, 1, sk - w)

    kv_pairs = R // TR * nj
    wo_pairs = G * R // TR * dt // 4
    steps = 2 * nj // STEP

    def feed(g, step):
        sem = sems.at[jax.lax.rem(g, NSLOT)]

        @pl.when(g < G)
        def _():
            feed_kv(g * R, kv_pairs * step // steps, kv_pairs * (step + 1) // steps, sem)

        @pl.when(g >= G)
        def _():
            for i in range(wo_pairs * step // steps, wo_pairs * (step + 1) // steps):
                a, b = (2 * i, 2 * i + 1) if PAIR else (i, wo_pairs + i)
                tile(wo_hbm, wob, (g - G) * (G // 2 * R), a, sem, 0)
                tile(wo_hbm, wob, (g - G) * (G // 2 * R), b, sem, 1)

    small = [pltpu.make_async_copy(x_hbm, xb, msem.at[0]),
             pltpu.make_async_copy(b1_hbm, b1b, msem.at[0]),
             pltpu.make_async_copy(b2_hbm, b2b, msem.at[0])]

    @pl.loop(0, d // TR)
    def _(r):
        for c in range(G * RT // 2):
            a, b = (2 * c, 2 * c + 1) if PAIRQ else (c, G * RT // 2 + c)
            tile(wq_hbm, wqb, r * TR, a, msem.at[1], 0)
            tile(wq_hbm, wqb, r * TR, b, msem.at[1], 1)

    for c in small:
        c.start()
    for g in range(NSLOT - 1):
        pl.loop(g * R // TR, (g + 1) * R // TR)(
            lambda r: feed_kv(r * TR, 0, nj, sems.at[g]))
    for c in small:
        c.wait()
    wait(wqb, msem.at[1])
    zero_s[...] = jnp.zeros(zero_s.shape, I32)

    def mlp(x, streaming):
        xn = _lhs(_layernorm(x))
        b1 = b1b[...].astype(F32)
        b2 = b2b[...].astype(F32)
        if streaming:
            wait(w1b, msem.at[0])
        h = jnp.concatenate(
            [_dot(xn, ld(w1w, t)) + b1[t:t + 1] for t in range(ft)], axis=1)
        h = _lhs(jax.nn.gelu(h, approximate=True))
        y = jnp.concatenate([b2[t:t + 1] for t in range(dt)], axis=1)
        cuts = (0, W2S, f) if streaming else (0, f)
        for i, (a, b) in enumerate(zip(cuts, cuts[1:])):
            if streaming:
                wait(w2b.at[:, a:b], msem.at[1 + i])
            y = y + jnp.concatenate(
                [_dot(h[:, a:b], ld(w2w, t, a, b - a)) for t in range(dt)], axis=1)
        return x + y

    x = jnp.broadcast_to(xb[0].astype(F32), (8, d))
    xn = _lhs(_layernorm(x))

    @pl.loop(0, G)
    def _(g):
        rows = pl.ds(pl.multiple_of(g * R, R), R)
        wait(kb.at[:, rows], sems.at[jax.lax.rem(g, NSLOT)])
        wait(vb.at[:, rows], sems.at[jax.lax.rem(g, NSLOT)])
        half = pl.ds(pl.multiple_of(g * (R // 2), R // 2), R // 2)
        kg, vg, qg = kw.at[:, half], vw.at[:, half], wqw.at[pl.ds(g * RT, RT)]
        q = _lhs(_own_head(jnp.concatenate(
            [_dot(xn, ld(qg, t)) for t in range(RT)], axis=1)))
        scores = []
        for j in range(nj):
            if j % STEP == 0:
                feed(g + NSLOT - 1, j // STEP)
            scores.append(_dot(q, ld(kg, j)))
        p, l = _softmax_terms(scores)
        o = jnp.zeros((8, R), F32)
        for j in range(nj):
            if j % STEP == 0:
                feed(g + NSLOT - 1, (nj + j) // STEP)
            o = o + _dot(_lhs(p[j]), ld(vg, j), True)
        o_s[g] = _lhs(_own_head(o / l))

    for i in range(f // TR * dt):
        tile(w1_hbm, w1b, 0, i, msem.at[0], 0)
        tile(w2_hbm, w2b, 0, i, msem.at[1 if i < W2S // TR * dt else 2], 1)

    attn = jnp.zeros((8, d), F32)
    for i in range(2):
        wait(wob.at[:, pl.ds(i * G // 2 * R, G // 2 * R)], sems.at[(G + i) % NSLOT])

        def out_proj(g, attn):
            og = wow.at[:, pl.ds(pl.multiple_of(g * (R // 2), R // 2), R // 2)]
            return attn + jnp.concatenate(
                [_dot(o_s[g], ld(og, t)) for t in range(dt)], axis=1)
        attn = jax.lax.fori_loop(i * G // 2, (i + 1) * G // 2, out_proj, attn)
    x = mlp(x + jnp.sum(attn, axis=0, keepdims=True), True)

    xn = _lhs(_layernorm(x))
    never = zero_s[...] != 0
    attn = jnp.zeros((8, d), F32)
    q, soft, pv = {}, {}, {}
    for s in range(-1, (G + 2) if NL else -1):
        do_q, do_k, do_v, do_o = s + 1 < G, 0 <= s < G, 1 <= s <= G, s >= 2
        cm = MXU_SHARE[s - 1] * nj // 32 if do_v else 0
        lane_sums = []
        if do_v:
            p = soft[s - 1][0]
            for u in range(R // 16):
                h = u * 16 // DH
                terms = [ld(vw, j, (s - 1) * R + u * 16, 16).astype(F32) * p[j][h:h + 1]
                         for j in range(nj - cm)]
                acc = terms[:3]
                for j in range(3, nj - cm):
                    acc[j % 3] = acc[j % 3] + terms[j]
                lane_sums.append((acc[0] + acc[1] + acc[2]).astype(BF))

        mxu_cost = (do_k * nj * R + do_q * RT * d + do_o * (dt + 2) * R + cm * 2 * R) * (
            1.0 if do_k else 0.97)
        done = [0, 0]

        def paced(a, cost):
            upto = min(len(lane_sums), int(len(lane_sums) * done[0] / mxu_cost))
            done[0] += cost
            if upto > done[1]:
                tie = pltpu.bitcast(lane_sums[done[1]], I32)
                for t in lane_sums[done[1] + 1:upto]:
                    tie = tie | pltpu.bitcast(t, I32)
                done[1] = upto
                a = pltpu.bitcast(jnp.where(never, tie, pltpu.bitcast(a, I32)), BF)
            return a

        def dot(a, b, trans=False):
            tiles = range(0, b.shape[0], LANES)
            if trans:
                return jnp.concatenate(
                    [_dot(paced(a, 2 * LANES), b[t:t + LANES], True) for t in tiles], axis=1)
            return _dot(jnp.concatenate(
                [paced(a[:, t:t + LANES], LANES) for t in tiles], axis=1), b)

        def out_proj():
            return jnp.concatenate(
                [dot(o, ld(wow, t, (s - 2) * R, R)) for t in range(dt)], axis=1)

        if do_o:
            o = dot(jnp.ones((16, LANES), BF), pv[s - 2][0], True) + pv[s - 2][1]
            o = _lhs(_own_head(o / soft[s - 2][1]))
        if do_k:
            soft[s] = _softmax_terms([dot(q[s], ld(kw, j, s * R, R)) for j in range(nj)])
        if do_v:
            rest = jnp.zeros((8, R), F32)
            for j in range(nj - cm, nj):
                if do_o and not do_k and j == nj - cm + 2:
                    attn, do_o = attn + out_proj(), False
                rest = rest + dot(_lhs(p[j]), ld(vw, j, (s - 1) * R, R), True)
            pv[s - 1] = (jnp.concatenate(lane_sums, axis=0), rest)
        if do_o:
            attn = attn + out_proj()
        if do_q:
            q[s + 1] = _lhs(_own_head(jnp.concatenate(
                [dot(xn, ld(wqw, (s + 1) * RT + t)) for t in range(RT)], axis=1)))

    if NL:
        x = mlp(x + jnp.sum(attn, axis=0, keepdims=True), False)
    o_ref[0] = x[0:1].astype(o_ref.dtype)


@jax.jit
def pallas_interleave_layers__sliding_block_cached__dense_activation_gelu__decode_kernel(
    A_x: jax.Array,
    A_k_cache: jax.Array,
    A_v_cache: jax.Array,
    A_wq: jax.Array,
    A_wo: jax.Array,
    B_x: jax.Array,
    B_w1: jax.Array,
    B_b1: jax.Array,
    B_w2: jax.Array,
    B_b2: jax.Array,
):
    del B_x
    d = A_x.shape[-1]
    sk = A_k_cache.shape[2]
    f = B_w1.shape[1]
    w = min(4096, max(256, sk // 4))
    nj, dt, ft = w // LANES, d // LANES, f // LANES
    kt = jnp.swapaxes(A_k_cache, 2, 3).reshape(HQ * DH, sk)
    vt = jnp.swapaxes(A_v_cache, 2, 3).reshape(HQ * DH, sk)

    def body(*refs):
        _kernel(*refs, sk=sk, w=w)

    return pl.pallas_call(
        body,
        out_shape=jax.ShapeDtypeStruct(A_x.shape, A_x.dtype),
        in_specs=[pl.BlockSpec(memory_space=pltpu.HBM)] * 9,
        out_specs=pl.BlockSpec(memory_space=pltpu.VMEM),
        scratch_shapes=[
            pltpu.VMEM(A_x.shape, BF),
            pltpu.VMEM((ft, LANES), BF),
            pltpu.VMEM((dt, LANES), BF),
            pltpu.VMEM((nj, HQ * DH // 2 + 8, LANES), I32),
            pltpu.VMEM((nj, HQ * DH // 2 + 8, LANES), I32),
            pltpu.VMEM((HQ * DH // LANES, d // 2, LANES), I32),
            pltpu.VMEM((dt, HQ * DH // 2, LANES), I32),
            pltpu.VMEM((ft, d // 2, LANES), I32),
            pltpu.VMEM((dt, f // 2, LANES), I32),
            pltpu.VMEM((G, 16, R), BF),
            pltpu.VMEM((8, LANES), I32),
            pltpu.SemaphoreType.DMA((NSLOT,)),
            pltpu.SemaphoreType.DMA((3,)),
        ],
        compiler_params=pltpu.CompilerParams(vmem_limit_bytes=126 * 1024 * 1024),
    )(A_x, kt, vt, A_wq, A_wo, B_w1, B_b1.reshape(ft, LANES), B_w2,
      B_b2.reshape(dt, LANES))
```

```python
import jax
import jax.numpy as jnp
import numpy as np
import jax.experimental.pallas as pl
import jax.experimental.pallas.tpu as pltpu

BF = jnp.bfloat16
F32 = jnp.float32
I32 = jnp.int32
LANES = 128
HQ, DH = 32, 192
HG = 4
G = HQ // HG
R = HG * DH
RT = R // LANES
NSLOT = 3
PAIR = 0
PAIRQ = 0
NL = 1
TR = 128
STEP = 4
W2S = 1280
SPLIT = 3
PACE = 1.0
PACEL = 0.97
MXU_SHARE = [int(c) for c in '3,2,2,2,2,2,3,12'.split(',')]
EXP2_SCALE = float(DH ** -0.5 * np.log2(np.e))


def _layernorm(x):
    m = jnp.mean(x, axis=-1, keepdims=True)
    c = x - m
    v = jnp.mean(c * c, axis=-1, keepdims=True)
    return c / jnp.sqrt(v + 1e-5)


def _lhs(x):
    return pltpu.bitcast(pltpu.bitcast(jnp.concatenate([x, x], axis=0).astype(BF), I32), BF)


def _dot(a, b, trans=False):
    return jax.lax.dot_general(a, b, (((1,), (1 if trans else 0,)), ((), ())),
                               preferred_element_type=F32)[:8]


def _own_head(x):
    r = jax.lax.broadcasted_iota(I32, (8, R), 0)
    c = jax.lax.broadcasted_iota(I32, (8, R), 1)
    return jnp.where((c >= r * DH) & (c < (r + 1) * DH), x, 0.0)


def _softmax_terms(scores):
    m = scores[0]
    for s in scores[1:]:
        m = jnp.maximum(m, s)
    m = jnp.max(m, axis=1, keepdims=True)
    p = [jnp.exp2((s - m) * EXP2_SCALE) for s in scores]
    l = p[0]
    for pj in p[1:]:
        l = l + pj
    return p, jnp.sum(l, axis=1, keepdims=True)


def _kernel(x_hbm, k_hbm, v_hbm, wq_hbm, wo_hbm, w1_hbm, b1_hbm, w2_hbm, b2_hbm,
            o_ref, xb, b1b, b2b, kw, vw, wqw, wow, w1w, w2w, o_s, zero_s, sems, msem,
            *, sk, w):
    nj = w // LANES
    dt = wow.shape[0]
    ft = w1w.shape[0]
    d, f = dt * LANES, ft * LANES
    kb, vb, wqb, wob, w1b, w2b = (r.bitcast(BF) for r in (kw, vw, wqw, wow, w1w, w2w))

    def ld(ref, t, r0=None, n=None):
        return pltpu.bitcast(ref[t] if r0 is None else ref[t, r0 // 2:(r0 + n) // 2], BF)

    def tile(src, dst, r0, i, sem, queue, c0=0):
        r, c = divmod(i, dst.shape[0])
        r = pl.ds(pl.multiple_of(r0 + r * TR, TR), TR)
        pltpu.make_async_copy(src.at[r, pl.ds(c0 + c * LANES, LANES)],
                              dst.at[c, r], sem).start(priority=queue)

    def wait(buf, sem):
        pltpu.make_async_copy(buf, buf, sem).wait()

    def feed_kv(r0, lo, hi, sem):
        for i in range(lo, hi):
            tile(k_hbm, kb, r0, i, sem, 0, sk - w)
            tile(v_hbm, vb, r0, i, sem, 1, sk - w)

    kv_pairs = R // TR * nj
    wo_pairs = G * R // TR * dt // 4
    steps = 2 * nj // STEP

    def feed(g, step):
        sem = sems.at[jax.lax.rem(g, NSLOT)]

        @pl.when(g < G)
        def _():
            feed_kv(g * R, kv_pairs * step // steps, kv_pairs * (step + 1) // steps, sem)

        @pl.when(g >= G)
        def _():
            for i in range(wo_pairs * step // steps, wo_pairs * (step + 1) // steps):
                a, b = (2 * i, 2 * i + 1) if PAIR else (i, wo_pairs + i)
                tile(wo_hbm, wob, (g - G) * (G // 2 * R), a, sem, 0)
                tile(wo_hbm, wob, (g - G) * (G // 2 * R), b, sem, 1)

    small = [pltpu.make_async_copy(x_hbm, xb, msem.at[0]),
             pltpu.make_async_copy(b1_hbm, b1b, msem.at[0]),
             pltpu.make_async_copy(b2_hbm, b2b, msem.at[0])]

    @pl.loop(0, d // TR)
    def _(r):
        for c in range(G * RT // 2):
            a, b = (2 * c, 2 * c + 1) if PAIRQ else (c, G * RT // 2 + c)
            tile(wq_hbm, wqb, r * TR, a, msem.at[1], 0)
            tile(wq_hbm, wqb, r * TR, b, msem.at[1], 1)

    for c in small:
        c.start()
    for g in range(NSLOT - 1):
        pl.loop(g * R // TR, (g + 1) * R // TR)(
            lambda r: feed_kv(r * TR, 0, nj, sems.at[g]))
    for c in small:
        c.wait()
    wait(wqb, msem.at[1])
    zero_s[...] = jnp.zeros(zero_s.shape, I32)

    def mlp(x, streaming):
        xn = _lhs(_layernorm(x))
        b1 = b1b[...].astype(F32)
        b2 = b2b[...].astype(F32)
        if streaming:
            wait(w1b, msem.at[0])
        h = jnp.concatenate(
            [_dot(xn, ld(w1w, t)) + b1[t:t + 1] for t in range(ft)], axis=1)
        h = _lhs(jax.nn.gelu(h, approximate=True))
        y = jnp.concatenate([b2[t:t + 1] for t in range(dt)], axis=1)
        cuts = (0, W2S, f) if streaming else (0, f)
        for i, (a, b) in enumerate(zip(cuts, cuts[1:])):
            if streaming:
                wait(w2b.at[:, a:b], msem.at[1 + i])
            y = y + jnp.concatenate(
                [_dot(h[:, a:b], ld(w2w, t, a, b - a)) for t in range(dt)], axis=1)
        return x + y

    x = jnp.broadcast_to(xb[0].astype(F32), (8, d))
    xn = _lhs(_layernorm(x))

    @pl.loop(0, G)
    def _(g):
        rows = pl.ds(pl.multiple_of(g * R, R), R)
        wait(kb.at[:, rows], sems.at[jax.lax.rem(g, NSLOT)])
        wait(vb.at[:, rows], sems.at[jax.lax.rem(g, NSLOT)])
        half = pl.ds(pl.multiple_of(g * (R // 2), R // 2), R // 2)
        kg, vg, qg = kw.at[:, half], vw.at[:, half], wqw.at[pl.ds(g * RT, RT)]
        q = _lhs(_own_head(jnp.concatenate(
            [_dot(xn, ld(qg, t)) for t in range(RT)], axis=1)))
        scores = []
        for j in range(nj):
            if j % STEP == 0:
                feed(g + NSLOT - 1, j // STEP)
            scores.append(_dot(q, ld(kg, j)))
        p, l = _softmax_terms(scores)
        o = jnp.zeros((8, R), F32)
        for j in range(nj):
            if j % STEP == 0:
                feed(g + NSLOT - 1, (nj + j) // STEP)
            o = o + _dot(_lhs(p[j]), ld(vg, j), True)
        o_s[g] = _lhs(_own_head(o / l))

    for i in range(f // TR * dt):
        tile(w1_hbm, w1b, 0, i, msem.at[0], 0)
        tile(w2_hbm, w2b, 0, i, msem.at[1 if i < W2S // TR * dt else 2], 1)

    attn = jnp.zeros((8, d), F32)
    for i in range(2):
        wait(wob.at[:, pl.ds(i * G // 2 * R, G // 2 * R)], sems.at[(G + i) % NSLOT])

        def out_proj(g, attn):
            og = wow.at[:, pl.ds(pl.multiple_of(g * (R // 2), R // 2), R // 2)]
            return attn + jnp.concatenate(
                [_dot(o_s[g], ld(og, t)) for t in range(dt)], axis=1)
        attn = jax.lax.fori_loop(i * G // 2, (i + 1) * G // 2, out_proj, attn)
    x = mlp(x + jnp.sum(attn, axis=0, keepdims=True), True)

    xn = _lhs(_layernorm(x))
    never = zero_s[...] != 0
    attn = jnp.zeros((8, d), F32)
    q, soft, pv = {}, {}, {}
    for s in range(-1, (G + 2) if NL else -1):
        do_q, do_k, do_v, do_o = s + 1 < G, 0 <= s < G, 1 <= s <= G, s >= 2
        cm = MXU_SHARE[s - 1] * nj // 32 if do_v else 0
        lane_sums = []
        if do_v:
            p = soft[s - 1][0]
            for u in range(R // 16):
                h = u * 16 // DH
                acc = []
                for j in range(nj - cm):
                    t = ld(vw, j, (s - 1) * R + u * 16, 16).astype(F32) * p[j][h:h + 1]
                    if j < SPLIT:
                        acc.append(t)
                    else:
                        acc[j % SPLIT] = acc[j % SPLIT] + t
                for t in acc[1:]:
                    acc[0] = acc[0] + t
                lane_sums.append(pltpu.bitcast(acc[0].astype(BF), I32))

        mxu_cost = (do_k * nj * R + do_q * RT * d + do_o * (dt + 2) * R + cm * 2 * R) * (
            PACE if do_k else PACEL)
        done = [0, 0]

        def paced(a, cost):
            upto = min(len(lane_sums), int(len(lane_sums) * done[0] / mxu_cost))
            done[0] += cost
            if upto > done[1]:
                tie = lane_sums[done[1]]
                for t in lane_sums[done[1] + 1:upto]:
                    tie = tie | t
                done[1] = upto
                a = pltpu.bitcast(jnp.where(never, tie, pltpu.bitcast(a, I32)), BF)
            return a

        def dot(a, b, trans=False):
            tiles = range(0, b.shape[0], LANES)
            if trans:
                return jnp.concatenate(
                    [_dot(paced(a, 2 * LANES), b[t:t + LANES], True) for t in tiles], axis=1)
            return _dot(jnp.concatenate(
                [paced(a[:, t:t + LANES], LANES) for t in tiles], axis=1), b)

        def out_proj():
            return jnp.concatenate(
                [dot(o, ld(wow, t, (s - 2) * R, R)) for t in range(dt)], axis=1)

        if do_o:
            o = dot(jnp.ones((16, LANES), BF), pv[s - 2][0], True) + pv[s - 2][1]
            o = _lhs(_own_head(o / soft[s - 2][1]))
        if do_k:
            soft[s] = _softmax_terms([dot(q[s], ld(kw, j, s * R, R)) for j in range(nj)])
        if do_v:
            rest = jnp.zeros((8, R), F32)
            for j in range(nj - cm, nj):
                if do_o and not do_k and j == nj - cm + 2:
                    attn, do_o = attn + out_proj(), False
                rest = rest + dot(_lhs(p[j]), ld(vw, j, (s - 1) * R, R), True)
            pv[s - 1] = (pltpu.bitcast(jnp.concatenate(lane_sums, axis=0), BF), rest)
        if do_o:
            attn = attn + out_proj()
        if do_q:
            q[s + 1] = _lhs(_own_head(jnp.concatenate(
                [dot(xn, ld(wqw, (s + 1) * RT + t)) for t in range(RT)], axis=1)))

    if NL:
        x = mlp(x + jnp.sum(attn, axis=0, keepdims=True), False)
    o_ref[0] = x[0:1].astype(o_ref.dtype)


@jax.jit
def pallas_interleave_layers__sliding_block_cached__dense_activation_gelu__decode_kernel(
    A_x: jax.Array,
    A_k_cache: jax.Array,
    A_v_cache: jax.Array,
    A_wq: jax.Array,
    A_wo: jax.Array,
    B_x: jax.Array,
    B_w1: jax.Array,
    B_b1: jax.Array,
    B_w2: jax.Array,
    B_b2: jax.Array,
):
    del B_x
    d = A_x.shape[-1]
    sk = A_k_cache.shape[2]
    f = B_w1.shape[1]
    w = min(4096, max(256, sk // 4))
    nj, dt, ft = w // LANES, d // LANES, f // LANES
    kt = jnp.swapaxes(A_k_cache, 2, 3).reshape(HQ * DH, sk)
    vt = jnp.swapaxes(A_v_cache, 2, 3).reshape(HQ * DH, sk)

    def body(*refs):
        _kernel(*refs, sk=sk, w=w)

    return pl.pallas_call(
        body,
        out_shape=jax.ShapeDtypeStruct(A_x.shape, A_x.dtype),
        in_specs=[pl.BlockSpec(memory_space=pltpu.HBM)] * 9,
        out_specs=pl.BlockSpec(memory_space=pltpu.VMEM),
        scratch_shapes=[
            pltpu.VMEM(A_x.shape, BF),
            pltpu.VMEM((ft, LANES), BF),
            pltpu.VMEM((dt, LANES), BF),
            pltpu.VMEM((nj, HQ * DH // 2 + 8, LANES), I32),
            pltpu.VMEM((nj, HQ * DH // 2 + 8, LANES), I32),
            pltpu.VMEM((HQ * DH // LANES, d // 2, LANES), I32),
            pltpu.VMEM((dt, HQ * DH // 2, LANES), I32),
            pltpu.VMEM((ft, d // 2, LANES), I32),
            pltpu.VMEM((dt, f // 2, LANES), I32),
            pltpu.VMEM((G, 16, R), BF),
            pltpu.VMEM((8, LANES), I32),
            pltpu.SemaphoreType.DMA((NSLOT,)),
            pltpu.SemaphoreType.DMA((3,)),
        ],
        compiler_params=pltpu.CompilerParams(vmem_limit_bytes=126 * 1024 * 1024, disable_bounds_checks=bool(E("NOBC", 0))),
    )(A_x, kt, vt, A_wq, A_wo, B_w1, B_b1.reshape(ft, LANES), B_w2,
      B_b2.reshape(dt, LANES))
```

```python
import jax
import jax.numpy as jnp
import numpy as np
import jax.experimental.pallas as pl
import jax.experimental.pallas.tpu as pltpu

BF = jnp.bfloat16
F32 = jnp.float32
I32 = jnp.int32
LANES = 128
HQ, DH = 32, 192
HG = 4
G = HQ // HG
R = HG * DH
RT = R // LANES
NSLOT = 3
PAIR = 0
PAIRQ = 0
NL = 1
TR = 128
STEP = 4
W2S = 1280
CK = 10
KB = 96
K0 = 3000
PACE0 = 1.0
NU = 7
VLIM = 127
NP = 3
NPL = 2
BOTH = 0
SPLIT = 2
PACE = 1.0
PACEL = 0.97
MXU_SHARE = [int(c) for c in '5,3,3,3,3,3,5,17'.split(',')]
EXP2_SCALE = float(DH ** -0.5 * np.log2(np.e))


def _layernorm(x):
    m = jnp.mean(x, axis=-1, keepdims=True)
    c = x - m
    v = jnp.mean(c * c, axis=-1, keepdims=True)
    return c / jnp.sqrt(v + 1e-5)


def _lhs(x):
    return pltpu.bitcast(pltpu.bitcast(jnp.concatenate([x, x], axis=0).astype(BF), I32), BF)


def _dot(a, b, trans=False):
    return jax.lax.dot_general(a, b, (((1,), (1 if trans else 0,)), ((), ())),
                               preferred_element_type=F32)[:8]


def _own_head(x):
    r = jax.lax.broadcasted_iota(I32, (8, R), 0)
    c = jax.lax.broadcasted_iota(I32, (8, R), 1)
    return jnp.where((c >= r * DH) & (c < (r + 1) * DH), x, 0.0)


def _softmax_terms(scores):
    m = scores[0]
    for s in scores[1:]:
        m = jnp.maximum(m, s)
    m = jnp.max(m, axis=1, keepdims=True)
    p = [jnp.exp2((s - m) * EXP2_SCALE) for s in scores]
    l = p[0]
    for pj in p[1:]:
        l = l + pj
    return p, jnp.sum(l, axis=1, keepdims=True)


def _kernel(x_hbm, k_hbm, v_hbm, wq_hbm, wo_hbm, w1_hbm, b1_hbm, w2_hbm, b2_hbm,
            o_ref, xb, b1b, b2b, kw, vw, wqw, wow, w1w, w2w, vu, o_s, zero_s, sems, msem,
            *, sk, w):
    nj = w // LANES
    dt = wow.shape[0]
    ft = w1w.shape[0]
    d, f = dt * LANES, ft * LANES
    kb, vb, wqb, wob, w1b, w2b = (r.bitcast(BF) for r in (kw, vw, wqw, wow, w1w, w2w))

    def ld(ref, t, r0=None, n=None):
        return pltpu.bitcast(ref[t] if r0 is None else ref[t, r0 // 2:(r0 + n) // 2], BF)

    def tile(src, dst, r0, i, sem, queue, c0=0):
        r, c = divmod(i, dst.shape[0])
        r = pl.ds(pl.multiple_of(r0 + r * TR, TR), TR)
        pltpu.make_async_copy(src.at[r, pl.ds(c0 + c * LANES, LANES)],
                              dst.at[c, r], sem).start(priority=queue)

    def wait(buf, sem):
        pltpu.make_async_copy(buf, buf, sem).wait()

    def feed_kv(r0, lo, hi, sem):
        for i in range(lo, hi):
            tile(k_hbm, kb, r0, i, sem, 0, sk - w)
            tile(v_hbm, vb, r0, i, sem, 1, sk - w)

    kv_pairs = R // TR * nj
    wo_pairs = G * R // TR * dt // 4
    steps = 2 * nj // STEP

    def feed(g, step):
        sem = sems.at[jax.lax.rem(g, NSLOT)]

        @pl.when(g < G)
        def _():
            feed_kv(g * R, kv_pairs * step // steps, kv_pairs * (step + 1) // steps, sem)

        @pl.when(g >= G)
        def _():
            for i in range(wo_pairs * step // steps, wo_pairs * (step + 1) // steps):
                a, b = (2 * i, 2 * i + 1) if PAIR else (i, wo_pairs + i)
                tile(wo_hbm, wob, (g - G) * (G // 2 * R), a, sem, 0)
                tile(wo_hbm, wob, (g - G) * (G // 2 * R), b, sem, 1)

    small = [pltpu.make_async_copy(x_hbm, xb, msem.at[0]),
             pltpu.make_async_copy(b1_hbm, b1b, msem.at[0]),
             pltpu.make_async_copy(b2_hbm, b2b, msem.at[0])]

    @pl.loop(0, d // TR)
    def _(r):
        for c in range(G * RT // 2):
            a, b = (2 * c, 2 * c + 1) if PAIRQ else (c, G * RT // 2 + c)
            tile(wq_hbm, wqb, r * TR, a, msem.at[1], 0)
            tile(wq_hbm, wqb, r * TR, b, msem.at[1], 1)

    for c in small:
        c.start()
    for g in range(NSLOT - 1):
        pl.loop(g * R // TR, (g + 1) * R // TR)(
            lambda r: feed_kv(r * TR, 0, nj, sems.at[g]))
    for c in small:
        c.wait()
    wait(wqb, msem.at[1])
    zero_s[...] = jnp.zeros(zero_s.shape, I32)

    def mlp(x, streaming):
        xn = _lhs(_layernorm(x))
        b1 = b1b[...].astype(F32)
        b2 = b2b[...].astype(F32)
        if streaming:
            wait(w1b, msem.at[0])
        h = jnp.concatenate(
            [_dot(xn, ld(w1w, t)) + b1[t:t + 1] for t in range(ft)], axis=1)
        h = _lhs(jax.nn.gelu(h, approximate=True))
        y = jnp.concatenate([b2[t:t + 1] for t in range(dt)], axis=1)
        cuts = (0, W2S, f) if streaming else (0, f)
        for i, (a, b) in enumerate(zip(cuts, cuts[1:])):
            if streaming:
                wait(w2b.at[:, a:b], msem.at[1 + i])
            y = y + jnp.concatenate(
                [_dot(h[:, a:b], ld(w2w, t, a, b - a)) for t in range(dt)], axis=1)
        return x + y

    x = jnp.broadcast_to(xb[0].astype(F32), (8, d))
    xn = _lhs(_layernorm(x))

    @pl.loop(0, G)
    def _(g):
        rows = pl.ds(pl.multiple_of(g * R, R), R)
        wait(kb.at[:, rows], sems.at[jax.lax.rem(g, NSLOT)])
        wait(vb.at[:, rows], sems.at[jax.lax.rem(g, NSLOT)])
        half = pl.ds(pl.multiple_of(g * (R // 2), R // 2), R // 2)
        kg, vg, qg = kw.at[:, half], vw.at[:, half], wqw.at[pl.ds(g * RT, RT)]
        q = _lhs(_own_head(jnp.concatenate(
            [_dot(xn, ld(qg, t)) for t in range(RT)], axis=1)))
        cm = MXU_SHARE[0]
        for i in range(1, G):
            cm = jnp.where(g == G - 1 - i, MXU_SHARE[i], cm)
        scores = []
        for j in range(nj):
            if j % STEP == 0:
                feed(g + NSLOT - 1, j // STEP)
            scores.append(_dot(q, ld(kg, j)))
        p, l = _softmax_terms(scores)
        o = jnp.zeros((8, R), F32)
        for j in range(nj):
            if j % STEP == 0:
                feed(g + NSLOT - 1, (nj + j) // STEP)
            o = o + _dot(_lhs(p[j]), ld(vg, j), True)
            if j < NU:
                wide = ld(vg, j).astype(F32).reshape(R // 16, 2, 8, LANES)
                vg[j] = pltpu.bitcast(wide[:, 0].reshape(R // 2, LANES), I32)
                vu[j, half] = wide[:, 1].reshape(R // 2, LANES)
            if j % STEP == STEP - 1 and j >= nj - max(MXU_SHARE):
                @pl.loop(jnp.maximum(j + 1 - STEP, nj - cm), j + 1)
                def _(jj):
                    for t in range(0, R, LANES):
                        vg[jj, t // 2:(t + LANES) // 2] = pltpu.bitcast(ld(vg, jj, t, LANES).T, I32)
        o_s[g] = _lhs(_own_head(o / l))

    for i in range(f // TR * dt):
        tile(w1_hbm, w1b, 0, i, msem.at[0], 0)
        tile(w2_hbm, w2b, 0, i, msem.at[1 if i < W2S // TR * dt else 2], 1)

    attn = jnp.zeros((8, d), F32)
    for i in range(2):
        wait(wob.at[:, pl.ds(i * G // 2 * R, G // 2 * R)], sems.at[(G + i) % NSLOT])

        def out_proj(g, attn):
            og = wow.at[:, pl.ds(pl.multiple_of(g * (R // 2), R // 2), R // 2)]
            return attn + jnp.concatenate(
                [_dot(o_s[g], ld(og, t)) for t in range(dt)], axis=1)
        attn = jax.lax.fori_loop(i * G // 2, (i + 1) * G // 2, out_proj, attn)
    x = mlp(x + jnp.sum(attn, axis=0, keepdims=True), True)

    xn = _lhs(_layernorm(x))
    never = zero_s[...] != 0
    attn = jnp.zeros((8, d), F32)
    q, soft, pv = {}, {}, {}
    for s in range(-1, (G + 2) if NL else -1):
        do_q, do_k, do_v, do_o = s + 1 < G, 0 <= s < G, 1 <= s <= G, s >= 2
        cm = MXU_SHARE[s - 1] * nj // 32 if do_v else 0
        lane_sums, marks = [], []
        if do_v:
            p = soft[s - 1][0]
            n = nj - cm
            npass = NP if n > 24 else NPL
            for h in range(HG):
                carry = {}
                for ps in range(npass):
                    for u in range(DH // 16):
                        acc = [carry[u]] if ps else []
                        for i, j in enumerate(range(ps, n, npass)):
                            r0 = (G - s) * R + h * DH + u * 16
                            if j < NU:
                                t = jnp.concatenate([pltpu.bitcast(vw[j, r0 // 2:r0 // 2 + 8], F32),
                                                     vu[j, r0 // 2:r0 // 2 + 8]], axis=0)
                            else:
                                t = ld(vw, j, r0, 16).astype(F32)
                            t = t * p[j][h:h + 1]
                            if len(acc) < SPLIT:
                                acc.append(t)
                            else:
                                acc[i % SPLIT] = acc[i % SPLIT] + t
                        for t in acc[1:]:
                            acc[0] = acc[0] + t
                        carry[u] = acc[0]
                        if ps == npass - 1:
                            lane_sums.append(pltpu.bitcast(acc[0].astype(BF), I32))
                            marks.append(lane_sums[-1])
                        else:
                            mk = pltpu.bitcast(acc[0], I32)
                            marks.append(mk[:8] | mk[8:] if BOTH else mk[8:])

        extra_scores = []
        if s == 0 and CK:
            qc = jnp.concatenate(
                [jnp.broadcast_to(q_row[0:1, t:t + LANES], (LANES, LANES)).T
                 for t in range(0, R, LANES)], axis=0)
            row = jax.lax.broadcasted_iota(I32, (8, LANES), 0)
            extra_scores = [jnp.zeros((8, LANES), F32)] * CK
            for h in range(HG):
                carry = {}
                for r in range(h * DH, (h + 1) * DH, KB):
                    for i in range(CK):
                        for u in range(r, r + KB, 16):
                            t = ld(kw, nj - CK + i, (G - 1) * R + u, 16).astype(F32) * qc[u:u + 16]
                            carry[i] = carry[i] + t if i in carry else t
                        if r + KB == (h + 1) * DH:
                            extra_scores[i] = jnp.where(
                                row == h, jnp.sum(carry[i], axis=0, keepdims=True), extra_scores[i])
                            marks.append(pltpu.bitcast(extra_scores[i], I32))
                        else:
                            marks.append(pltpu.bitcast(carry[i][8:], I32))

        mxu_cost = (do_k * nj * R + do_q * RT * d + do_o * (dt + 2) * R + cm * R) * (
            PACE if do_k else PACEL)
        done = [0, 0]
        if extra_scores:
            mxu_cost = (nj - CK) * R * PACE0 - K0
            done[0] = -K0

        def paced(a, cost):
            upto = min(len(marks), int(len(marks) * done[0] / mxu_cost))
            done[0] += cost
            if upto > done[1]:
                tie = marks[done[1]]
                for t in marks[done[1] + 1:upto]:
                    tie = tie | t
                done[1] = upto
                a = pltpu.bitcast(jnp.where(never, tie, pltpu.bitcast(a, I32)), BF)
            return a

        def dot(a, b, trans=False):
            tiles = range(0, b.shape[0], LANES)
            if trans:
                return jnp.concatenate(
                    [_dot(paced(a, 2 * LANES), b[t:t + LANES], True) for t in tiles], axis=1)
            return _dot(jnp.concatenate(
                [paced(a[:, t:t + LANES], LANES) for t in tiles], axis=1), b)

        def out_proj():
            return jnp.concatenate(
                [dot(o, ld(wow, t, (G + 1 - s) * R, R)) for t in range(dt)], axis=1)

        if do_o:
            o = dot(jnp.ones((16, LANES), BF), pv[s - 2][0], True) + pv[s - 2][1]
            o = _lhs(_own_head(o / soft[s - 2][1]))
        if do_k:
            soft[s] = _softmax_terms([dot(q[s], ld(kw, j, (G - 1 - s) * R, R)) for j in range(nj - len(extra_scores))] + extra_scores)
        if do_v:
            rest = jnp.zeros((8, R), F32)
            for j in range(nj - cm, nj):
                if do_o and not do_k and j == nj - cm + 2:
                    attn, do_o = attn + out_proj(), False
                rest = rest + jnp.concatenate([dot(_lhs(p[j]), ld(vw, j, (G - s) * R + t, LANES)) for t in range(0, R, LANES)], axis=1)
            pv[s - 1] = (pltpu.bitcast(jnp.concatenate(lane_sums, axis=0), BF), rest)
        if do_o:
            attn = attn + out_proj()
        if do_q:
            q_row = jnp.concatenate(
                [dot(xn, ld(wqw, (G - 2 - s) * RT + t)) for t in range(RT)], axis=1)
            q[s + 1] = _lhs(_own_head(q_row))
            q_row = q_row.astype(BF).astype(F32)

    if NL:
        x = mlp(x + jnp.sum(attn, axis=0, keepdims=True), False)
    o_ref[0] = x[0:1].astype(o_ref.dtype)


@jax.jit
def pallas_interleave_layers__sliding_block_cached__dense_activation_gelu__decode_kernel(
    A_x: jax.Array,
    A_k_cache: jax.Array,
    A_v_cache: jax.Array,
    A_wq: jax.Array,
    A_wo: jax.Array,
    B_x: jax.Array,
    B_w1: jax.Array,
    B_b1: jax.Array,
    B_w2: jax.Array,
    B_b2: jax.Array,
):
    del B_x
    d = A_x.shape[-1]
    sk = A_k_cache.shape[2]
    f = B_w1.shape[1]
    w = min(4096, max(256, sk // 4))
    nj, dt, ft = w // LANES, d // LANES, f // LANES
    kt = jnp.swapaxes(A_k_cache, 2, 3).reshape(HQ * DH, sk)
    vt = jnp.swapaxes(A_v_cache, 2, 3).reshape(HQ * DH, sk)

    def body(*refs):
        _kernel(*refs, sk=sk, w=w)

    return pl.pallas_call(
        body,
        out_shape=jax.ShapeDtypeStruct(A_x.shape, A_x.dtype),
        in_specs=[pl.BlockSpec(memory_space=pltpu.HBM)] * 9,
        out_specs=pl.BlockSpec(memory_space=pltpu.VMEM),
        scratch_shapes=[
            pltpu.VMEM(A_x.shape, BF),
            pltpu.VMEM((ft, LANES), BF),
            pltpu.VMEM((dt, LANES), BF),
            pltpu.VMEM((nj, HQ * DH // 2 + 8, LANES), I32),
            pltpu.VMEM((nj, HQ * DH // 2 + 8, LANES), I32),
            pltpu.VMEM((HQ * DH // LANES, d // 2, LANES), I32),
            pltpu.VMEM((dt, HQ * DH // 2, LANES), I32),
            pltpu.VMEM((ft, d // 2, LANES), I32),
            pltpu.VMEM((dt, f // 2, LANES), I32),
            pltpu.VMEM((max(NU, 1), HQ * DH // 2 + 8, LANES), F32),
            pltpu.VMEM((G, 16, R), BF),
            pltpu.VMEM((8, LANES), I32),
            pltpu.SemaphoreType.DMA((NSLOT,)),
            pltpu.SemaphoreType.DMA((3,)),
        ],
        compiler_params=pltpu.CompilerParams(vmem_limit_bytes=VLIM * 1024 * 1024, disable_bounds_checks=bool(E("NOBC", 0))),
    )(A_x, kt, vt, A_wq, A_wo, B_w1, B_b1.reshape(ft, LANES), B_w2,
      B_b2.reshape(dt, LANES))
```

```python
import jax
import jax.numpy as jnp
import numpy as np
import jax.experimental.pallas as pl
import jax.experimental.pallas.tpu as pltpu

BF = jnp.bfloat16
F32 = jnp.float32
I32 = jnp.int32
LANES = 128
HQ, DH = 32, 192
HG = 4
G = HQ // HG
R = HG * DH
RT = R // LANES
NSLOT = 3
STEP = 4
V_MXU = (17, 5, 3, 3, 3, 3, 3, 5)
V_WIDE = 7
K_VPU = 10
EXP2_SCALE = float(DH ** -0.5 * np.log2(np.e))


def _layernorm(x):
    m = jnp.mean(x, axis=-1, keepdims=True)
    c = x - m
    v = jnp.mean(c * c, axis=-1, keepdims=True)
    return c / jnp.sqrt(v + 1e-5)


def _lhs(x):
    return pltpu.bitcast(pltpu.bitcast(jnp.concatenate([x, x], axis=0).astype(BF), I32), BF)


def _dot(a, b, trans=False):
    return jax.lax.dot_general(a, b, (((1,), (1 if trans else 0,)), ((), ())),
                               preferred_element_type=F32)[:8]


def _wide(tiles):
    return jnp.concatenate(tiles, axis=1)


def _own_head(x):
    r = jax.lax.broadcasted_iota(I32, (8, R), 0)
    c = jax.lax.broadcasted_iota(I32, (8, R), 1)
    return jnp.where((c >= r * DH) & (c < (r + 1) * DH), x, 0.0)


def _softmax_terms(scores):
    m = scores[0]
    for s in scores[1:]:
        m = jnp.maximum(m, s)
    m = jnp.max(m, axis=1, keepdims=True)
    p = [jnp.exp2((s - m) * EXP2_SCALE) for s in scores]
    l = p[0]
    for pj in p[1:]:
        l = l + pj
    return p, jnp.sum(l, axis=1, keepdims=True)


def _kernel(x_hbm, k_hbm, v_hbm, wq_hbm, wo_hbm, w1_hbm, b1_hbm, w2_hbm, b2_hbm,
            o_ref, xb, b1b, b2b, kw, vw, wqw, wow, w1w, w2w, vu, o_s, zero_s,
            ksem, vsem, msem):
    nj, dt, ft = kw.shape[0], wow.shape[0], w1w.shape[0]
    d, f = dt * LANES, ft * LANES
    k0 = k_hbm.shape[1] - nj * LANES
    f_cut = f - 2 * LANES
    kb, vb, wqb, wob, w1b, w2b = (r.bitcast(BF) for r in (kw, vw, wqw, wow, w1w, w2w))

    def ld(ref, t, r0=None, n=None):
        return pltpu.bitcast(ref[t] if r0 is None else ref[t, r0 // 2:(r0 + n) // 2], BF)

    def tile(src, dst, r0, i, sem, queue, c0=0):
        r, c = divmod(i, dst.shape[0])
        r = pl.ds(pl.multiple_of(r0 + r * LANES, LANES), LANES)
        pltpu.make_async_copy(src.at[r, pl.ds(c0 + c * LANES, LANES)],
                              dst.at[c, r], sem).start(priority=queue)

    def wait(buf, sem):
        pltpu.make_async_copy(buf, buf, sem).wait()

    def feed_kv(r0, lo, hi, slot):
        for i in range(lo, hi):
            tile(k_hbm, kb, r0, i, ksem.at[slot], 0, k0)
            tile(v_hbm, vb, r0, i, vsem.at[slot], 1, k0)

    def feed(g, step):
        slot = jax.lax.rem(g, NSLOT)
        steps = 2 * nj // STEP

        @pl.when(g < G)
        def _():
            n = RT * nj
            feed_kv(g * R, n * step // steps, n * (step + 1) // steps, slot)

        @pl.when(g >= G)
        def _():
            n = G * RT * dt // 4
            for i in range(n * step // steps, n * (step + 1) // steps):
                tile(wo_hbm, wob, (g - G) * (G // 2 * R), i, ksem.at[slot], 0)
                tile(wo_hbm, wob, (g - G) * (G // 2 * R), n + i, ksem.at[slot], 1)

    @pl.loop(0, dt)
    def _(r):
        for c in range(G * RT):
            tile(wq_hbm, wqb, r * LANES, c, msem.at[1], c % 2)

    small = [pltpu.make_async_copy(x_hbm, xb, msem.at[0]),
             pltpu.make_async_copy(b1_hbm, b1b, msem.at[0]),
             pltpu.make_async_copy(b2_hbm, b2b, msem.at[0])]
    for c in small:
        c.start()
    for g in range(NSLOT - 1):
        pl.loop(g * RT, (g + 1) * RT)(lambda r, g=g: feed_kv(r * LANES, 0, nj, g))
    for c in small:
        c.wait()
    wait(wqb, msem.at[1])
    zero_s[...] = jnp.zeros(zero_s.shape, I32)

    def mlp(x, streaming):
        xn = _lhs(_layernorm(x))
        b1 = b1b[...].astype(F32)
        b2 = b2b[...].astype(F32)
        if streaming:
            wait(w1b, msem.at[0])
        h = _wide([_dot(xn, ld(w1w, t)) + b1[t:t + 1] for t in range(ft)])
        h = _lhs(jax.nn.gelu(h, approximate=True))
        y = _wide([b2[t:t + 1] for t in range(dt)])
        cuts = (0, f_cut, f) if streaming else (0, f)
        for i, (a, b) in enumerate(zip(cuts, cuts[1:])):
            if streaming:
                wait(w2b.at[:, a:b], msem.at[1 + i])
            y = y + _wide([_dot(h[:, a:b], ld(w2w, t, a, b - a)) for t in range(dt)])
        return x + y

    x = jnp.broadcast_to(xb[0].astype(F32), (8, d))
    xn = _lhs(_layernorm(x))

    @pl.loop(0, G)
    def _(g):
        rows = pl.ds(pl.multiple_of(g * R, R), R)
        wait(kb.at[:, rows], ksem.at[jax.lax.rem(g, NSLOT)])
        wait(vb.at[:, rows], vsem.at[jax.lax.rem(g, NSLOT)])
        half = pl.ds(pl.multiple_of(g * (R // 2), R // 2), R // 2)
        kg, vg, qg = kw.at[:, half], vw.at[:, half], wqw.at[pl.ds(g * RT, RT)]
        q = _lhs(_own_head(_wide([_dot(xn, ld(qg, t)) for t in range(RT)])))
        scores = []
        for j in range(nj):
            if j % STEP == 0:
                feed(g + NSLOT - 1, j // STEP)
            scores.append(_dot(q, ld(kg, j)))
        p, l = _softmax_terms(scores)

        v_mxu = V_MXU[0]
        for i in range(1, G):
            v_mxu = jnp.where(g == i, V_MXU[i], v_mxu)
        o = jnp.zeros((8, R), F32)
        for j in range(nj):
            if j % STEP == 0:
                feed(g + NSLOT - 1, (nj + j) // STEP)
            o = o + _dot(_lhs(p[j]), ld(vg, j), True)
            if j < V_WIDE:
                v32 = ld(vg, j).astype(F32).reshape(R // 16, 2, 8, LANES)
                vg[j] = pltpu.bitcast(v32[:, 0].reshape(R // 2, LANES), I32)
                vu[j, half] = v32[:, 1].reshape(R // 2, LANES)
            if j % STEP == STEP - 1 and j >= nj - max(V_MXU):
                @pl.loop(jnp.maximum(j + 1 - STEP, nj - v_mxu), j + 1)
                def _(jj):
                    for t in range(0, R, LANES):
                        vg[jj, t // 2:(t + LANES) // 2] = pltpu.bitcast(
                            ld(vg, jj, t, LANES).T, I32)
        o_s[g] = _lhs(_own_head(o / l))

    for i in range(ft * dt):
        tile(w1_hbm, w1b, 0, i, msem.at[0], 0)
        tile(w2_hbm, w2b, 0, i, msem.at[1 if i < f_cut // LANES * dt else 2], 1)

    def out_proj(g, attn):
        og = wow.at[:, pl.ds(pl.multiple_of(g * (R // 2), R // 2), R // 2)]
        return attn + _wide([_dot(o_s[g], ld(og, t)) for t in range(dt)])

    attn = jnp.zeros((8, d), F32)
    for i in range(2):
        wait(wob.at[:, pl.ds(i * G // 2 * R, G // 2 * R)], ksem.at[(G + i) % NSLOT])
        attn = jax.lax.fori_loop(i * G // 2, (i + 1) * G // 2, out_proj, attn)
    x = mlp(x + jnp.sum(attn, axis=0, keepdims=True), True)

    def vpu_scores(g, q_row, marks):
        q_row = q_row[0:1].astype(BF).astype(F32)
        q_col = jnp.concatenate(
            [jnp.broadcast_to(q_row[:, t:t + LANES], (LANES, LANES)).T
             for t in range(0, R, LANES)], axis=0)
        row = jax.lax.broadcasted_iota(I32, (8, LANES), 0)
        out = [jnp.zeros((8, LANES), F32)] * K_VPU
        for h in range(HG):
            acc = {}
            for r0 in (h * DH, h * DH + DH // 2):
                for i in range(K_VPU):
                    for r in range(r0, r0 + DH // 2, 16):
                        t = ld(kw, nj - K_VPU + i, g * R + r, 16).astype(F32) * q_col[r:r + 16]
                        acc[i] = acc[i] + t if i in acc else t
                    if r0 == h * DH:
                        marks.append(pltpu.bitcast(acc[i][8:], I32))
                    else:
                        out[i] = jnp.where(
                            row == h, jnp.sum(acc[i], axis=0, keepdims=True), out[i])
                        marks.append(pltpu.bitcast(out[i], I32))
        return out

    def vpu_pv(g, p, marks):
        n = nj - V_MXU[g]
        passes = 3 if n > 24 else 2
        out = []
        for h in range(HG):
            part = {}
            for ps in range(passes):
                for r in range(g * R + h * DH, g * R + (h + 1) * DH, 16):
                    acc = [part[r]] if ps else []
                    for i, j in enumerate(range(ps, n, passes)):
                        if j < V_WIDE:
                            v = jnp.concatenate(
                                [pltpu.bitcast(vw[j, r // 2:r // 2 + 8], F32),
                                 vu[j, r // 2:r // 2 + 8]], axis=0)
                        else:
                            v = ld(vw, j, r, 16).astype(F32)
                        t = v * p[j][h:h + 1]
                        if len(acc) < 2:
                            acc.append(t)
                        else:
                            acc[i % 2] = acc[i % 2] + t
                    part[r] = acc[0] + acc[1]
                    if ps < passes - 1:
                        marks.append(pltpu.bitcast(part[r][8:], I32))
                    else:
                        out.append(pltpu.bitcast(part[r].astype(BF), I32))
                        marks.append(out[-1])
        return pltpu.bitcast(jnp.concatenate(out, axis=0), BF)

    xn = _lhs(_layernorm(x))
    never = zero_s[...] != 0
    attn = jnp.zeros((8, d), F32)
    q, soft, pv = {}, {}, {}
    for g in range(G, -3, -1):
        do_q, do_k, do_v, do_o = (0 <= i < G for i in range(g - 1, g + 3))
        marks, late_scores = [], []
        done = [0, 0]
        if do_v:
            p = soft[g + 1][0]
            lane_sums = vpu_pv(g + 1, p, marks)
            mxu_rows = R * (do_k * nj + do_q * dt + do_o * (dt + 2) + V_MXU[g + 1])
        elif do_k:
            late_scores = vpu_scores(g, q[g], marks)
            done[0] = -4 * R
            mxu_rows = R * (nj - K_VPU - 4)

        def paced(a, cost):
            upto = min(len(marks), int(len(marks) * done[0] / mxu_rows)) if marks else 0
            done[0] += cost
            if upto > done[1]:
                tie = marks[done[1]]
                for t in marks[done[1] + 1:upto]:
                    tie = tie | t
                done[1] = upto
                a = pltpu.bitcast(jnp.where(never, tie, pltpu.bitcast(a, I32)), BF)
            return a

        def dot(a, b):
            return _dot(_wide([paced(a[:, t:t + LANES], LANES)
                               for t in range(0, b.shape[0], LANES)]), b)

        def wo_dot():
            return _wide([dot(o, ld(wow, t, (g + 2) * R, R)) for t in range(dt)])

        if do_o:
            ones = jnp.ones((16, LANES), BF)
            o = _wide([_dot(paced(ones, 2 * LANES), pv[g + 2][0][t:t + LANES], True)
                       for t in range(0, R, LANES)]) + pv[g + 2][1]
            o = _lhs(_own_head(o / soft[g + 2][1]))
        if do_k:
            q_heads = _lhs(_own_head(q[g]))
            soft[g] = _softmax_terms(
                [dot(q_heads, ld(kw, j, g * R, R)) for j in range(nj - len(late_scores))]
                + late_scores)
        if do_v:
            rest = jnp.zeros((8, R), F32)
            for i, j in enumerate(range(nj - V_MXU[g + 1], nj)):
                if do_o and not do_k and i == 2:
                    attn, do_o = attn + wo_dot(), False
                pj = _lhs(p[j])
                rest = rest + _wide([dot(pj, ld(vw, j, (g + 1) * R + t, LANES))
                                     for t in range(0, R, LANES)])
            pv[g + 1] = (lane_sums, rest)
        if do_o:
            attn = attn + wo_dot()
        if do_q:
            q[g - 1] = _wide([dot(xn, ld(wqw, (g - 1) * RT + t)) for t in range(RT)])

    x = mlp(x + jnp.sum(attn, axis=0, keepdims=True), False)
    o_ref[0] = x[0:1].astype(o_ref.dtype)


@jax.jit
def pallas_interleave_layers__sliding_block_cached__dense_activation_gelu__decode_kernel(
    A_x: jax.Array,
    A_k_cache: jax.Array,
    A_v_cache: jax.Array,
    A_wq: jax.Array,
    A_wo: jax.Array,
    B_x: jax.Array,
    B_w1: jax.Array,
    B_b1: jax.Array,
    B_w2: jax.Array,
    B_b2: jax.Array,
):
    del B_x
    d = A_x.shape[-1]
    sk = A_k_cache.shape[2]
    f = B_w1.shape[1]
    w = min(4096, max(256, sk // 4))
    nj, dt, ft = w // LANES, d // LANES, f // LANES
    assert V_WIDE + max(V_MXU) <= nj
    kt = jnp.swapaxes(A_k_cache, 2, 3).reshape(HQ * DH, sk)
    vt = jnp.swapaxes(A_v_cache, 2, 3).reshape(HQ * DH, sk)
    kv_rows = HQ * DH // 2 + 8

    return pl.pallas_call(
        _kernel,
        out_shape=jax.ShapeDtypeStruct(A_x.shape, A_x.dtype),
        in_specs=[pl.BlockSpec(memory_space=pltpu.HBM)] * 9,
        out_specs=pl.BlockSpec(memory_space=pltpu.VMEM),
        scratch_shapes=[
            pltpu.VMEM(A_x.shape, BF),
            pltpu.VMEM((ft, LANES), BF),
            pltpu.VMEM((dt, LANES), BF),
            pltpu.VMEM((nj, kv_rows, LANES), I32),
            pltpu.VMEM((nj, kv_rows, LANES), I32),
            pltpu.VMEM((G * RT, d // 2, LANES), I32),
            pltpu.VMEM((dt, HQ * DH // 2, LANES), I32),
            pltpu.VMEM((ft, d // 2, LANES), I32),
            pltpu.VMEM((dt, f // 2, LANES), I32),
            pltpu.VMEM((V_WIDE, kv_rows, LANES), F32),
            pltpu.VMEM((G, 16, R), BF),
            pltpu.VMEM((8, LANES), I32),
            pltpu.SemaphoreType.DMA((NSLOT,)),
            pltpu.SemaphoreType.DMA((NSLOT,)),
            pltpu.SemaphoreType.DMA((3,)),
        ],
        compiler_params=pltpu.CompilerParams(vmem_limit_bytes=127 * 1024 * 1024),
    )(A_x, kt, vt, A_wq, A_wo, B_w1, B_b1.reshape(ft, LANES), B_w2,
      B_b2.reshape(dt, LANES))
```
